```python
import jax
import jax.numpy as jnp

def _softmax(x, axis=-1):
    return jax.nn.softmax(x, axis=axis)
def _gelu(x):
    return jax.nn.gelu(x, approximate=True)
def _silu(x):
    return jax.nn.silu(x)
def _sigmoid(x):
    return jax.nn.sigmoid(x)
def _layernorm(x, axis=-1, eps=1e-5):
    m = jnp.mean(x, axis=axis, keepdims=True)
    v = jnp.var(x, axis=axis, keepdims=True)
    return (x - m) / jnp.sqrt(v + eps)
def _scatter_add(tgt, idx, src, axis=0):
    return tgt.at[idx].add(src)
def _segment_sum(src, seg, n):
    return jax.ops.segment_sum(src, seg, n)
class _Rng:
    def __init__(self, key):
        self._k = key
    def _next(self):
        self._k, sub = jax.random.split(self._k)
        return sub
    def normal(self, shape):
        return jax.random.normal(self._next(), shape, dtype=jnp.bfloat16)
    def randint(self, lo, hi, shape):
        return jax.random.randint(self._next(), shape, lo, hi, dtype=jnp.int32)
    def uniform(self, shape, lo=0.0, hi=1.0):
        return jax.random.uniform(self._next(), shape, jnp.bfloat16, lo, hi)
    def permutation(self, n):
        return jax.random.permutation(self._next(), n)


kernel_name = 'gated_mix__gqa_block_cached__dense_activation_relu__decode'

def _fwd_setup_inputs():
    _rng = _Rng(jax.random.key(int.from_bytes(__import__("os").urandom(4), "little")))
    _w = (lambda a: (lambda t: t.astype(jnp.bfloat16) if jnp.issubdtype(t.dtype, jnp.floating) else t)(jnp.asarray(a)))
    def _A_setup():
        B, Sq, D = 2, 1, 512
        Hq, Hkv, Sk, Dh = 32, 8, 8192, 128
        assert Hq % Hkv == 0, (Hq, Hkv)
        return {
            "x": _w((lambda *s: _rng.normal(s) * 0.05)(B, Sq, D)),
            "k_cache": _w((lambda *s: _rng.normal(s) * 0.05)(B, Hkv, Sk, Dh)),
            "v_cache": _w((lambda *s: _rng.normal(s) * 0.05)(B, Hkv, Sk, Dh)),
            "wq": _w((lambda *s: _rng.normal(s) * 0.05)(D, Hq * Dh) * (D ** -0.5)),
            "wo": _w((lambda *s: _rng.normal(s) * 0.05)(Hq * Dh, D) * ((Hq * Dh) ** -0.5)),
        }
    _A_in = _A_setup()

    def _B_setup():
        B, S, D, Dff = 2, 1, 512, 1792
        return {
            "x": _w((lambda *s: _rng.normal(s) * 0.05)(B, S, D)),
            "w1": _w((lambda *s: _rng.normal(s) * 0.05)(D, Dff)),
            "w2": _w((lambda *s: _rng.normal(s) * 0.05)(Dff, D)),
        }
    _B_in = _B_setup()

    return {
        "A_x": _A_in["x"],
        "A_k_cache": _A_in["k_cache"],
        "A_v_cache": _A_in["v_cache"],
        "A_wq": _A_in["wq"],
        "A_wo": _A_in["wo"],
        "B_x": _B_in["x"],
        "B_w1": _B_in["w1"],
        "B_w2": _B_in["w2"],
        "gate_w": _w((lambda *s: _rng.normal(s) * 0.05)(512)),
    }

def _fwd_reference(A_x, A_k_cache, A_v_cache, A_wq, A_wo, B_x, B_w1, B_w2, gate_w):
    def _A_ref(x, k_cache, v_cache, wq, wo):
        B, Sq, D = x.shape
        Hq, Dh = 32, 128
        Hkv = k_cache.shape[1]
        rep = Hq // Hkv
        q = (lambda x, *d: x.transpose(*d))((x @ wq).reshape(B, Sq, Hq, Dh), 0, 2, 1, 3)
        k = jnp.repeat(k_cache, rep, axis=1)
        v = jnp.repeat(v_cache, rep, axis=1)
        scores = jnp.einsum("bhqd,bhkd->bhqk", q, k) * (Dh ** -0.5)
        p = _softmax(scores, axis=-1)
        o = jnp.einsum("bhqk,bhkd->bhqd", p, v)
        return (lambda x, *d: x.transpose(*d))(o, 0, 2, 1, 3).reshape(B, Sq, Hq * Dh) @ wo

    def _B_ref(x, w1, w2):
        h = jnp.einsum("bsd,df->bsf", x, w1)
        zero = jnp.zeros_like(h)
        h = jnp.maximum(h, zero)
        return jnp.einsum("bsf,fd->bsd", h, w2)

    x = A_x
    g = _sigmoid((x * gate_w).sum(-1, keepdims=True))
    a = _A_ref(x, A_k_cache, A_v_cache, A_wq, A_wo)
    b = _B_ref(x, B_w1, B_w2)
    return g * a + (1 - g) * b


def setup_inputs():
    _inp = _fwd_setup_inputs()
    _gk = jax.random.fold_in(jax.random.key(int.from_bytes(__import__("os").urandom(4), "little")), 2**31 - 1)
    _shapes = [[2, 1, 512]]
    _dtypes = ['bfloat16']
    _gks = jax.random.split(_gk, len(_shapes))
    _gs = [jax.random.normal(k, s, dtype=jnp.dtype(d)) * 0.05 for k, s, d in zip(_gks, _shapes, _dtypes)]
    _inp["grad_out"] = _gs[0]
    return _inp

def reference(A_x, A_k_cache, A_v_cache, A_wq, A_wo, B_w1, B_w2, gate_w, B_x, grad_out):
    _const = dict(B_x=B_x)
    def _f(*_d):
        return _fwd_reference(**{'A_x': _d[0], 'A_k_cache': _d[1], 'A_v_cache': _d[2], 'A_wq': _d[3], 'A_wo': _d[4], 'B_w1': _d[5], 'B_w2': _d[6], 'gate_w': _d[7], **_const})
    _out, _vjp = jax.vjp(_f, A_x, A_k_cache, A_v_cache, A_wq, A_wo, B_w1, B_w2, gate_w)
    _grads = _vjp(grad_out)
    _out0 = jnp.asarray(_out)
    return (_out0, *[jnp.asarray(_g) for _g in _grads])
```

```python
import jax
import jax.numpy as jnp
from jax import lax
import jax.experimental.pallas as pl
import jax.experimental.pallas.tpu as pltpu

BF16 = jnp.bfloat16
F32 = jnp.float32
_NN = (((1,), (0,)), ((), ()))
_NT = (((1,), (1,)), ((), ()))
_TN = (((0,), (0,)), ((), ()))

HQ, DH = 32, 128
SEG = 128
SEGS = 32
SWITCH = 13
CHUNK = 2048


def _dot(a, b, dims):
    return lax.dot_general(a, b, dims, preferred_element_type=F32)


def _rows01(ref):
    v = ref[...].astype(F32)
    return jnp.concatenate([v, jnp.zeros((8 - v.shape[0], v.shape[1]), F32)], axis=0)


def _kernel(
    x_hbm, k_hbm, v_hbm, wq_hbm, wo_hbm, w1_hbm, w2_hbm, gw_hbm, go_hbm,
    out_hbm, dx_hbm, dk_hbm, dv_hbm, dwq_hbm, dwo_hbm, dw1_hbm, dw2_hbm, dgw_hbm,
    kbuf, vbuf, wq_v, wo_v, w1_v, w2_v, dwq_v, dwo_v, dw1_v, dw2_v,
    x_v, go_v, gw_v, out_v, dx_v, dgw_v,
    qq_s, dd_s, od_s, s_s, dp_s, pd_s,
    small_sem, wq_sem, wo_sem, ffn_sem, kv_sem, out_sem,
):
    nh, sk, _ = k_hbm.shape
    hkv = nh // 2
    rep = HQ // hkv
    scale = DH ** -0.5
    nchunk = sk // CHUNK

    small = [
        pltpu.make_async_copy(src, dst, small_sem)
        for src, dst in ((x_hbm, x_v), (go_hbm, go_v), (gw_hbm, gw_v))
    ]
    wq_in = pltpu.make_async_copy(wq_hbm, wq_v, wq_sem)
    wo_in = pltpu.make_async_copy(wo_hbm, wo_v, wo_sem)
    ffn_in = [
        pltpu.make_async_copy(w1_hbm, w1_v, ffn_sem),
        pltpu.make_async_copy(w2_hbm, w2_v, ffn_sem),
    ]

    def kv_in(i):
        return (
            pltpu.make_async_copy(k_hbm.at[i], kbuf.at[i + 1], kv_sem.at[i]),
            pltpu.make_async_copy(v_hbm.at[i], vbuf.at[i + 1], kv_sem.at[i]),
        )

    wq_in.start()
    for c in small:
        c.start()
    wo_in.start()

    @pl.loop(0, nh)
    def _(i):
        for c in kv_in(i):
            c.start()

    for c in ffn_in:
        c.start()

    for c in small:
        c.wait()
    x = _rows01(x_v)
    go = _rows01(go_v)
    gw = gw_v[...].astype(F32).reshape(1, -1)
    gate = jax.nn.sigmoid(jnp.sum(x * gw, axis=-1, keepdims=True))
    x_b = x.astype(BF16)
    da_b = (gate * go).astype(BF16)

    def to_heads(dst, val):
        for b in range(2):
            for h in range(hkv):
                for r in range(rep):
                    c0 = (h * rep + r) * DH
                    piece = val[b:b + 1, c0:c0 + DH]
                    dst[b * hkv + h, r:r + 1, :] = piece
                    dst[b * hkv + h, r + rep:r + rep + 1, :] = piece

    wq_in.wait()
    to_heads(qq_s, _dot(x_b, wq_v[...], _NN))
    wo_in.wait()
    to_heads(dd_s, _dot(da_b, wo_v[...], _NT))

    def cache_out(buf, hbm, half, j):
        n = hkv * sk // (SEG * SEGS)
        src = buf.at[pl.ds(half * hkv, hkv)].reshape(n, SEGS, SEG, DH)
        return pltpu.make_async_copy(src.at[:, j], hbm.at[half, :, j], out_sem)

    def start_cache_out(half):
        for buf, hbm in ((kbuf, dk_hbm), (vbuf, dv_hbm)):
            @pl.loop(0, SEGS)
            def _(j):
                cache_out(buf, hbm, half, j).start()

    top = lax.broadcasted_iota(jnp.int32, (8, DH), 0) < rep

    @pl.loop(0, nh)
    def _(i):
        @pl.when(i == SWITCH)
        def _():
            for c in ffn_in:
                c.wait()
            start_cache_out(0)

        for c in kv_in(i):
            c.wait()
        qq = qq_s[i]
        dd = dd_s[i]
        qq_b = qq.astype(BF16)
        dd_b = dd.astype(BF16)

        @pl.loop(0, nchunk)
        def _(c):
            rows = pl.ds(pl.multiple_of(c * CHUNK, CHUNK), CHUNK)
            s_s[c] = _dot(qq_b, kbuf[i + 1, rows, :], _NT) * scale
            dp_s[c] = _dot(dd_b, vbuf[i + 1, rows, :], _NT)

        s = s_s[...]
        m = jnp.max(jnp.max(s, axis=0), axis=-1, keepdims=True)
        e = jnp.exp(s - m)
        inv = 1.0 / jnp.sum(jnp.sum(e, axis=0), axis=-1, keepdims=True)
        p = e * inv
        dp = dp_s[...]
        delta = jnp.sum(jnp.sum(p * dp, axis=0), axis=-1, keepdims=True)
        ds = p * (dp - delta) * scale
        upper = lax.broadcasted_iota(jnp.int32, p.shape, 1) < rep
        pd_s[...] = jnp.where(upper, p, ds)

        rhs = jnp.concatenate(
            [jnp.where(top, dd, 0.0), jnp.where(top, 0.0, qq)], axis=1
        ).astype(BF16)

        def pass2(c, acc):
            rows = pl.ds(pl.multiple_of(c * CHUNK, CHUNK), CHUNK)
            pd = pd_s[c].astype(BF16)
            o = _dot(pd, vbuf[i + 1, rows, :], _NN)
            dq = _dot(pd, kbuf[i + 1, rows, :], _NN)
            g = _dot(pd, rhs, _TN).astype(BF16)
            vbuf[i, rows, :] = g[:, :DH]
            kbuf[i, rows, :] = g[:, DH:]
            return acc + jnp.where(top, o, dq)

        od_s[i] = lax.fori_loop(0, nchunk, pass2, jnp.zeros((8, DH), F32))

    db_b = ((1.0 - gate) * go).astype(BF16)
    h = _dot(x_b, w1_v[...], _NN)
    hr_b = jnp.maximum(h, 0.0).astype(BF16)
    b_out = _dot(hr_b, w2_v[...], _NN)
    slope = jnp.where(h > 0.0, 1.0, jnp.where(h == 0.0, 0.5, 0.0))
    dh_b = (_dot(db_b, w2_v[...], _NT) * slope).astype(BF16)
    dw2_v[...] = _dot(hr_b, db_b, _TN).astype(BF16)
    dw1_v[...] = _dot(x_b, dh_b, _TN).astype(BF16)

    def from_heads(r0):
        row = lax.broadcasted_iota(jnp.int32, (8, DH), 0)
        cols = []
        for hh in range(hkv):
            for r in range(rep):
                a0 = jnp.broadcast_to(od_s[hh, r0 + r:r0 + r + 1, :], (8, DH))
                a1 = jnp.broadcast_to(od_s[hkv + hh, r0 + r:r0 + r + 1, :], (8, DH))
                cols.append(jnp.where(row == 0, a0, jnp.where(row == 1, a1, 0.0)))
        return jnp.concatenate(cols, axis=1).astype(BF16)

    o_b = from_heads(0)
    dq_b = from_heads(rep)
    a_out = _dot(o_b, wo_v[...], _NN)
    out = gate * a_out + (1.0 - gate) * b_out
    dz = jnp.sum(go * (a_out - b_out), axis=-1, keepdims=True) * gate * (1.0 - gate)
    dx = _dot(dq_b, wq_v[...], _NT) + _dot(dh_b, w1_v[...], _NT) + dz * gw
    dgw = jnp.sum(dz * x, axis=0, keepdims=True)
    out_v[...] = out[:2].astype(BF16)
    dx_v[...] = dx[:2].astype(BF16)
    dgw_v[...] = dgw.astype(BF16).reshape(-1)
    dwo_v[...] = _dot(o_b, da_b, _TN).astype(BF16)
    dwq_v[...] = _dot(x_b, dq_b, _TN).astype(BF16)

    rest = [
        pltpu.make_async_copy(src, dst, out_sem)
        for src, dst in (
            (out_v, out_hbm), (dx_v, dx_hbm), (dgw_v, dgw_hbm),
            (dw1_v, dw1_hbm), (dw2_v, dw2_hbm), (dwq_v, dwq_hbm), (dwo_v, dwo_hbm),
        )
    ]
    for c in rest:
        c.start()
    start_cache_out(1)

    for c in rest:
        c.wait()
    for buf in (kbuf, vbuf):
        whole = buf.at[pl.ds(0, nh)]
        pltpu.make_async_copy(whole, whole, out_sem).wait()


@jax.jit
def pallas_gated_mix__gqa_block_cached__dense_activation_relu__decode_kernel(
    A_x: jax.Array,
    A_k_cache: jax.Array,
    A_v_cache: jax.Array,
    A_wq: jax.Array,
    A_wo: jax.Array,
    B_x: jax.Array,
    B_w1: jax.Array,
    B_w2: jax.Array,
    gate_w: jax.Array,
    grad_out: jax.Array,
):
    del B_x
    nb, hkv, sk, dh = A_k_cache.shape
    nh = nb * hkv
    rows = lambda a: a.reshape(nb, a.shape[-1])
    x2 = rows(A_x)
    cache_out = (nb, hkv * sk // (SEG * SEGS), SEGS, SEG, dh)
    like = lambda a: jax.ShapeDtypeStruct(a.shape, BF16)
    vmem = lambda a: pltpu.VMEM(a.shape, BF16)
    hbm = pl.BlockSpec(memory_space=pltpu.HBM)

    outs = pl.pallas_call(
        _kernel,
        out_shape=(
            like(x2), like(x2),
            jax.ShapeDtypeStruct(cache_out, BF16), jax.ShapeDtypeStruct(cache_out, BF16),
            like(A_wq), like(A_wo), like(B_w1), like(B_w2), like(gate_w),
        ),
        in_specs=[hbm] * 9,
        out_specs=(hbm,) * 9,
        scratch_shapes=[
            pltpu.VMEM((nh + 1, sk, dh), BF16), pltpu.VMEM((nh + 1, sk, dh), BF16),
            vmem(A_wq), vmem(A_wo), vmem(B_w1), vmem(B_w2),
            vmem(A_wq), vmem(A_wo), vmem(B_w1), vmem(B_w2),
            vmem(x2), vmem(x2), vmem(gate_w),
            vmem(x2), vmem(x2), vmem(gate_w),
            pltpu.VMEM((nh, 8, dh), F32), pltpu.VMEM((nh, 8, dh), F32),
            pltpu.VMEM((nh, 8, dh), F32),
            pltpu.VMEM((sk // CHUNK, 8, CHUNK), F32),
            pltpu.VMEM((sk // CHUNK, 8, CHUNK), F32),
            pltpu.VMEM((sk // CHUNK, 8, CHUNK), F32),
            pltpu.SemaphoreType.DMA, pltpu.SemaphoreType.DMA, pltpu.SemaphoreType.DMA,
            pltpu.SemaphoreType.DMA, pltpu.SemaphoreType.DMA((nh,)),
            pltpu.SemaphoreType.DMA,
        ],
        compiler_params=pltpu.CompilerParams(vmem_limit_bytes=120 * 1024 * 1024),
    )(
        x2, A_k_cache.reshape(nh, sk, dh), A_v_cache.reshape(nh, sk, dh), A_wq, A_wo,
        B_w1, B_w2, gate_w, rows(grad_out),
    )
    out, dx, dk, dv, dwq, dwo, dw1, dw2, dgw = outs
    return (
        out.reshape(A_x.shape), dx.reshape(A_x.shape),
        dk.reshape(A_k_cache.shape), dv.reshape(A_v_cache.shape),
        dwq, dwo, dw1, dw2, dgw,
    )
```

```python
import jax
import jax.numpy as jnp
from jax import lax
import jax.experimental.pallas as pl
import jax.experimental.pallas.tpu as pltpu

BF16 = jnp.bfloat16
F32 = jnp.float32
_NN = (((1,), (0,)), ((), ()))
_NT = (((1,), (1,)), ((), ()))
_TN = (((0,), (0,)), ((), ()))

HQ = 32
ROWS = 8
PIECE = 128
PIECES = 32
STEP = 16
GROUPS = (6, 6, 6, 7, 7)
SPLIT = 4
TURN = 13
TAIL = 448
QUEUE = 64
REFILL = 24


def _dot(a, b, dims):
    return lax.dot_general(a, b, dims, preferred_element_type=F32)


def _pad_rows(ref):
    v = ref[...].astype(F32)
    return jnp.concatenate([v, jnp.zeros((ROWS - v.shape[0], v.shape[1]), F32)], axis=0)


def _kernel(
    x_hbm, k_hbm, v_hbm, wq_hbm, wo_hbm, w1_hbm, w2_hbm, gw_hbm, go_hbm,
    out_hbm, dx_hbm, dk_hbm, dv_hbm, dwq_hbm, dwo_hbm, dw1_hbm, dw2_hbm, dgw_hbm,
    kbuf, vbuf, wq_v, wo_v, w1_v, w2_v, dwq_v, dwo_v, dw1_v, dw2_v,
    x_v, go_v, gw_v, out_v, dx_v, dgw_v,
    q_s, do_s, od_s, s_s, dp_s, pd_s,
    in_sem, kv_sem, out_sem,
):
    nb = x_hbm.shape[0]
    nh, _, dh = q_s.shape
    hkv = nh // nb
    rep = HQ // hkv
    assert 2 * rep == ROWS
    bph = k_hbm.shape[0] // nh
    steps = s_s.shape[0]
    scale = dh ** -0.5

    small_in = [
        pltpu.make_async_copy(src, dst, in_sem.at[0])
        for src, dst in ((x_hbm, x_v), (go_hbm, go_v), (gw_hbm, gw_v))
    ]
    wq_in = pltpu.make_async_copy(wq_hbm, wq_v, in_sem.at[1])
    wo_in = pltpu.make_async_copy(wo_hbm, wo_v, in_sem.at[2])
    head = pl.ds(0, w2_hbm.shape[0] - TAIL)
    tail = pl.ds(w2_hbm.shape[0] - TAIL, TAIL)
    ffn_in = [
        pltpu.make_async_copy(w1_hbm, w1_v, in_sem.at[3]),
        pltpu.make_async_copy(w2_hbm.at[head], w2_v.at[head], in_sem.at[3]),
    ]
    tail_in = pltpu.make_async_copy(w2_hbm.at[tail], w2_v.at[tail], in_sem.at[4])

    def kv_in(i):
        src, dst = pl.ds(i * bph, bph), pl.ds((i + 1) * bph, bph)
        return (
            pltpu.make_async_copy(k_hbm.at[src], kbuf.at[dst], kv_sem.at[i]),
            pltpu.make_async_copy(v_hbm.at[src], vbuf.at[dst], kv_sem.at[i]),
        )

    for copy in (wq_in, *small_in, wo_in):
        copy.start()

    @pl.loop(0, nh)
    def _(i):
        for copy in kv_in(i):
            copy.start()

    for copy in (*ffn_in, tail_in):
        copy.start()

    for copy in small_in:
        copy.wait()
    x = _pad_rows(x_v)
    go = _pad_rows(go_v)
    gw = gw_v[...].astype(F32).reshape(1, -1)
    gate = jax.nn.sigmoid(jnp.sum(x * gw, axis=-1, keepdims=True))
    x_b = x.astype(BF16)
    da_b = (gate * go).astype(BF16)

    def to_heads(dst, val):
        for b in range(nb):
            for hq in range(HQ):
                h, r = divmod(hq, rep)
                row = val[b:b + 1, hq * dh:(hq + 1) * dh]
                dst[b * hkv + h, r:r + 1, :] = row
                dst[b * hkv + h, r + rep:r + rep + 1, :] = row

    wq_in.wait()
    to_heads(q_s, _dot(x_b, wq_v[...], _NN))
    wo_in.wait()
    to_heads(do_s, _dot(da_b, wo_v[...], _NT))

    runs = []
    for g, n in enumerate(GROUPS):
        blocks = pl.ds(sum(GROUPS[:g]), n)
        runs += [(kbuf, dk_hbm, blocks, 0), (vbuf, dv_hbm, blocks, 1)]

    def start_cache_out(lo, hi):
        for r, (buf, hbm, blocks, sem) in enumerate(runs):
            first, last = max(lo - r * PIECES, 0), min(hi - r * PIECES, PIECES)
            if first < last:
                @pl.loop(first, last)
                def _(j):
                    pltpu.make_async_copy(
                        buf.at[blocks, j], hbm.at[blocks, j], out_sem.at[sem]
                    ).start()

    top = lax.broadcasted_iota(jnp.int32, (ROWS, dh), 0) < rep

    @pl.loop(0, nh)
    def _(i):
        @pl.when(i == TURN)
        def _():
            for copy in ffn_in:
                copy.wait()
            start_cache_out(0, QUEUE)

        for later in range(TURN + 1, nh):
            @pl.when(i == later)
            def _():
                lo = QUEUE + (later - TURN - 1) * REFILL
                start_cache_out(lo, lo + REFILL)

        for copy in kv_in(i):
            copy.wait()
        q = q_s[i]
        do = do_s[i]
        q_b = q.astype(BF16)
        do_b = do.astype(BF16)

        def part(slot, c):
            per_block = PIECES // STEP
            return slot * bph + c // per_block, pl.ds((c % per_block) * STEP, STEP)

        def load(buf, c):
            return buf[part(i + 1, c)].reshape(STEP * PIECE, dh)

        @pl.loop(0, steps)
        def _(c):
            s_s[c] = _dot(q_b, load(kbuf, c), _NT) * scale
            dp_s[c] = _dot(do_b, load(vbuf, c), _NT)

        s = s_s[...]
        m = jnp.max(jnp.max(s, axis=0), axis=-1, keepdims=True)
        e = jnp.exp(s - m)
        p = e * (1.0 / jnp.sum(jnp.sum(e, axis=0), axis=-1, keepdims=True))
        dp = dp_s[...]
        delta = jnp.sum(jnp.sum(p * dp, axis=0), axis=-1, keepdims=True)
        ds = p * (dp - delta) * scale
        pd_s[...] = jnp.where(lax.broadcasted_iota(jnp.int32, p.shape, 1) < rep, p, ds)
        rhs = jnp.concatenate(
            [jnp.where(top, do, 0.0), jnp.where(top, 0.0, q)], axis=1
        ).astype(BF16)

        def second_pass(c, acc):
            pd = pd_s[c].astype(BF16)
            o = _dot(pd, load(vbuf, c), _NN)
            dq = _dot(pd, load(kbuf, c), _NN)
            dvk = _dot(pd, rhs, _TN).astype(BF16)
            vbuf[part(i, c)] = dvk[:, :dh].reshape(STEP, PIECE, dh)
            kbuf[part(i, c)] = dvk[:, dh:].reshape(STEP, PIECE, dh)
            return acc + jnp.where(top, o, dq)

        od_s[i] = lax.fori_loop(0, steps, second_pass, jnp.zeros((ROWS, dh), F32))

    started = QUEUE + (nh - TURN - 1) * REFILL
    start_cache_out(started, started + REFILL)
    started += REFILL

    tail_in.wait()
    db_b = ((1.0 - gate) * go).astype(BF16)
    pre = _dot(x_b, w1_v[...], _NN)
    act_b = jnp.maximum(pre, 0.0).astype(BF16)
    b_out = _dot(act_b, w2_v[...], _NN)
    slope = jnp.where(pre > 0.0, 1.0, jnp.where(pre == 0.0, 0.5, 0.0))
    dpre_b = (_dot(db_b, w2_v[...], _NT) * slope).astype(BF16)
    dw2_v[...] = _dot(act_b, db_b, _TN).astype(BF16).reshape(dw2_v.shape)
    dw1_v[...] = _dot(x_b, dpre_b, _TN).astype(BF16).reshape(dw1_v.shape)

    start_cache_out(started, started + REFILL)
    started += REFILL

    def from_heads(r0):
        row = lax.broadcasted_iota(jnp.int32, (ROWS, dh), 0)
        cols = []
        for hq in range(HQ):
            h, r = divmod(hq, rep)
            col = jnp.zeros((ROWS, dh), F32)
            for b in range(nb):
                col = jnp.where(row == b, od_s[b * hkv + h, r0 + r:r0 + r + 1, :], col)
            cols.append(col)
        return jnp.concatenate(cols, axis=1).astype(BF16)

    o_b = from_heads(0)
    dq_b = from_heads(rep)
    a_out = _dot(o_b, wo_v[...], _NN)
    dz = jnp.sum(go * (a_out - b_out), axis=-1, keepdims=True) * gate * (1.0 - gate)
    out = gate * a_out + (1.0 - gate) * b_out
    dx = _dot(dq_b, wq_v[...], _NT) + _dot(dpre_b, w1_v[...], _NT) + dz * gw
    out_v[...] = out[:nb].astype(BF16)
    dx_v[...] = dx[:nb].astype(BF16)
    dgw_v[...] = jnp.sum(dz * x, axis=0, keepdims=True).astype(BF16).reshape(-1)
    dwo_v[...] = _dot(o_b, da_b, _TN).astype(BF16).reshape(dwo_v.shape)
    dwq_v[...] = _dot(x_b, dq_b, _TN).astype(BF16).reshape(dwq_v.shape)

    small_out = [
        pltpu.make_async_copy(src, dst, out_sem.at[2])
        for src, dst in ((out_v, out_hbm), (dx_v, dx_hbm), (dgw_v, dgw_hbm))
    ]
    for copy in small_out:
        copy.start()
    last_run = (len(runs) - 1) * PIECES
    start_cache_out(started, last_run)

    weights = ((dwq_v, dwq_hbm), (dwo_v, dwo_hbm), (dw1_v, dw1_hbm), (dw2_v, dw2_hbm))

    def start_weight_out(w, j, rows, c, cols):
        buf, hbm = weights[w]
        idx = slice(None), pl.ds(pl.multiple_of(j * rows, rows), rows), pl.ds(c * cols, cols)
        pltpu.make_async_copy(buf.at[idx], hbm.at[idx], out_sem.at[3 + w]).start()

    @pl.loop(0, dwq_v.shape[1] // 8)
    def _(j):
        for c in range(4):
            start_weight_out(0, j, 8, c, dwq_v.shape[2] // 4)
            start_weight_out(1, 4 * j + c, 16, 0, dwo_v.shape[2])

    @pl.loop(0, dw1_v.shape[1] // 8)
    def _(j):
        for c in range(2):
            start_weight_out(2, j, 8, c, dw1_v.shape[2] // 2)

            @pl.when(2 * j + c < dw2_v.shape[1] // 16)
            def _():
                start_weight_out(3, 2 * j + c, 16, 0, dw2_v.shape[2])

    start_cache_out(last_run, last_run + PIECES)

    for copy in small_out:
        copy.wait()
    for w, (buf, _) in enumerate(weights):
        pltpu.make_async_copy(buf, buf, out_sem.at[3 + w]).wait()
    for sem, buf in enumerate((kbuf, vbuf)):
        done = buf.at[pl.ds(0, nh * bph)]
        pltpu.make_async_copy(done, done, out_sem.at[sem]).wait()


@jax.jit
def pallas_gated_mix__gqa_block_cached__dense_activation_relu__decode_kernel(
    A_x: jax.Array,
    A_k_cache: jax.Array,
    A_v_cache: jax.Array,
    A_wq: jax.Array,
    A_wo: jax.Array,
    B_x: jax.Array,
    B_w1: jax.Array,
    B_w2: jax.Array,
    gate_w: jax.Array,
    grad_out: jax.Array,
):
    del B_x
    nb, hkv, sk, dh = A_k_cache.shape
    nh = nb * hkv
    rows = (nb, A_x.shape[-1])
    bph = sk // (PIECE * PIECES)
    cache = (nh * bph, PIECES, PIECE, dh)
    slots = ((nh + 1) * bph, PIECES, PIECE, dh)
    scores = (sk // (STEP * PIECE), ROWS, STEP * PIECE)
    weights = (A_wq, A_wo, B_w1, B_w2)
    split = [(SPLIT, w.shape[0] // SPLIT, w.shape[1]) for w in weights]
    assert sum(GROUPS) == cache[0]
    assert split[1][1] // 16 == 4 * (split[0][1] // 8)
    assert split[3][1] // 16 <= 2 * (split[2][1] // 8)

    out_shapes = (rows, rows, cache, cache, *split, gate_w.shape)
    hbm = pl.BlockSpec(memory_space=pltpu.HBM)
    outs = pl.pallas_call(
        _kernel,
        out_shape=tuple(jax.ShapeDtypeStruct(s, BF16) for s in out_shapes),
        in_specs=[hbm] * 9,
        out_specs=(hbm,) * 9,
        scratch_shapes=[
            *(pltpu.VMEM(s, BF16) for s in (slots, slots, *(w.shape for w in weights), *split)),
            *(pltpu.VMEM(s, BF16) for s in (rows, rows, gate_w.shape) * 2),
            *(pltpu.VMEM((nh, ROWS, dh), F32) for _ in range(3)),
            *(pltpu.VMEM(scores, F32) for _ in range(3)),
            pltpu.SemaphoreType.DMA((5,)),
            pltpu.SemaphoreType.DMA((nh,)),
            pltpu.SemaphoreType.DMA((7,)),
        ],
        compiler_params=pltpu.CompilerParams(
            vmem_limit_bytes=120 * 1024 * 1024,
            disable_bounds_checks=True,
            disable_semaphore_checks=True,
        ),
    )(
        A_x.reshape(rows), A_k_cache.reshape(cache), A_v_cache.reshape(cache),
        *weights, gate_w, grad_out.reshape(rows),
    )
    like = (A_x, A_x, A_k_cache, A_v_cache, *weights, gate_w)
    return tuple(o.reshape(a.shape) for o, a in zip(outs, like))
```

```python
import functools

import jax
import jax.numpy as jnp
from jax import lax
import jax.experimental.pallas as pl
import jax.experimental.pallas.tpu as pltpu

BF16 = jnp.bfloat16
F32 = jnp.float32
_NN = (((1,), (0,)), ((), ()))
_NT = (((1,), (1,)), ((), ()))
_TN = (((0,), (0,)), ((), ()))

HQ = 32
ROWS = 8
PIECE = 64
PIECES = 64
STEP = 32
GROUPS = (7, 7, 6, 6, 6)
SPLITS = (4, 4, 2, 2)
TURN = 12
TAIL = 384
QUEUE = 64
REFILL = 20


def _dot(a, b, dims):
    return lax.dot_general(a, b, dims, preferred_element_type=F32)


def _pad_rows(ref):
    v = ref[...].astype(F32)
    return jnp.concatenate([v, jnp.zeros((ROWS - v.shape[0], v.shape[1]), F32)], axis=0)


def _kernel(*refs, heads):
    dv_hbm, vbuf, dv_sem = refs[12], refs[19], refs[-1]
    pl.run_scoped(
        functools.partial(_streams, *refs),
        pltpu.SemaphoreType.DMA((5,)),
        pltpu.SemaphoreType.DMA((heads,)),
        pltpu.SemaphoreType.DMA((6,)),
    )
    pltpu.make_async_copy(vbuf.at[pl.ds(0, dv_hbm.shape[0])], dv_hbm, dv_sem).wait()


def _streams(
    x_hbm, k_hbm, v_hbm, wq_hbm, wo_hbm, w1_hbm, w2_hbm, gw_hbm, go_hbm,
    out_hbm, dx_hbm, dk_hbm, dv_hbm, dwq_hbm, dwo_hbm, dw1_hbm, dw2_hbm, dgw_hbm,
    kbuf, vbuf, wq_v, wo_v, w1_v, w2_v, dwq_v, dwo_v, dw1_v, dw2_v,
    x_v, go_v, gw_v, out_v, dx_v, dgw_v,
    q_s, do_s, od_s, s_s, dp_s, pd_s,
    dv_sem, in_sem, kv_sem, out_sem,
):
    nb = x_hbm.shape[0]
    nh, _, dh = q_s.shape
    hkv = nh // nb
    rep = HQ // hkv
    assert 2 * rep == ROWS
    bph = k_hbm.shape[0] // nh
    steps = s_s.shape[0]
    scale = dh ** -0.5

    small_in = [
        pltpu.make_async_copy(src, dst, in_sem.at[0])
        for src, dst in ((x_hbm, x_v), (go_hbm, go_v), (gw_hbm, gw_v))
    ]
    wq_in = pltpu.make_async_copy(wq_hbm, wq_v, in_sem.at[1])
    wo_in = pltpu.make_async_copy(wo_hbm, wo_v, in_sem.at[2])
    head = pl.ds(0, w2_hbm.shape[0] - TAIL)
    tail = pl.ds(w2_hbm.shape[0] - TAIL, TAIL)
    ffn_in = [
        pltpu.make_async_copy(w1_hbm, w1_v, in_sem.at[3]),
        pltpu.make_async_copy(w2_hbm.at[head], w2_v.at[head], in_sem.at[3]),
    ]
    tail_in = pltpu.make_async_copy(w2_hbm.at[tail], w2_v.at[tail], in_sem.at[4])

    def kv_in(i):
        src, dst = pl.ds(i * bph, bph), pl.ds((i + 1) * bph, bph)
        return (
            pltpu.make_async_copy(k_hbm.at[src], kbuf.at[dst], kv_sem.at[i]),
            pltpu.make_async_copy(v_hbm.at[src], vbuf.at[dst], kv_sem.at[i]),
        )

    for copy in (wq_in, *small_in, wo_in):
        copy.start()

    @pl.loop(0, nh)
    def _(i):
        for copy in kv_in(i):
            copy.start()

    for copy in (*ffn_in, tail_in):
        copy.start()

    for copy in small_in:
        copy.wait()
    x = _pad_rows(x_v)
    go = _pad_rows(go_v)
    gw = gw_v[...].astype(F32).reshape(1, -1)
    gate = jax.nn.sigmoid(jnp.sum(x * gw, axis=-1, keepdims=True))
    x_b = x.astype(BF16)
    da_b = (gate * go).astype(BF16)

    def to_heads(dst, val):
        for b in range(nb):
            for hq in range(HQ):
                h, r = divmod(hq, rep)
                row = val[b:b + 1, hq * dh:(hq + 1) * dh]
                dst[b * hkv + h, r:r + 1, :] = row
                dst[b * hkv + h, r + rep:r + rep + 1, :] = row

    wq_in.wait()
    to_heads(q_s, _dot(x_b, wq_v[...], _NN))
    wo_in.wait()
    to_heads(do_s, _dot(da_b, wo_v[...], _NT))

    runs = []
    for g, n in enumerate(GROUPS):
        blocks = pl.ds(sum(GROUPS[:g]), n)
        runs += [(kbuf, dk_hbm, blocks, out_sem.at[0]), (vbuf, dv_hbm, blocks, dv_sem)]

    def start_cache_out(lo, hi):
        for r, (buf, hbm, blocks, sem) in enumerate(runs):
            first, last = max(lo - r * PIECES, 0), min(hi - r * PIECES, PIECES)
            if first < last:
                @pl.loop(first, last)
                def _(j):
                    pltpu.make_async_copy(buf.at[blocks, j], hbm.at[blocks, j], sem).start()

    top = lax.broadcasted_iota(jnp.int32, (ROWS, dh), 0) < rep

    def refill(i, lo, hi):
        for later in range(TURN, nh):
            @pl.when(i == later)
            def _():
                base = QUEUE + 3 * REFILL * (later - TURN)
                start_cache_out(base + lo * REFILL, base + hi * REFILL)

    @pl.loop(0, nh)
    def _(i):
        @pl.when(i == TURN)
        def _():
            for copy in ffn_in:
                copy.wait()
            start_cache_out(0, QUEUE)

        for copy in kv_in(i):
            copy.wait()
        q = q_s[i]
        do = do_s[i]
        q_b = q.astype(BF16)
        do_b = do.astype(BF16)

        def part(slot, c):
            per_block = PIECES // STEP
            return slot * bph + c // per_block, pl.ds((c % per_block) * STEP, STEP)

        def load(buf, c):
            return buf[part(i + 1, c)].reshape(STEP * PIECE, dh)

        @pl.loop(0, steps)
        def _(c):
            s_s[c] = _dot(q_b, load(kbuf, c), _NT) * scale
            dp_s[c] = _dot(do_b, load(vbuf, c), _NT)

        s = s_s[...]
        m = jnp.max(jnp.max(s, axis=0), axis=-1, keepdims=True)
        e = jnp.exp(s - m)
        p = e * (1.0 / jnp.sum(jnp.sum(e, axis=0), axis=-1, keepdims=True))
        dp = dp_s[...]
        delta = jnp.sum(jnp.sum(p * dp, axis=0), axis=-1, keepdims=True)
        ds = p * (dp - delta) * scale
        pd_s[...] = jnp.where(lax.broadcasted_iota(jnp.int32, p.shape, 1) < rep, p, ds)
        rhs = jnp.concatenate(
            [jnp.where(top, do, 0.0), jnp.where(top, 0.0, q)], axis=1
        ).astype(BF16)

        refill(i, 0, 1)

        def second_pass(c, acc):
            pd = pd_s[c].astype(BF16)
            o = _dot(pd, load(vbuf, c), _NN)
            dq = _dot(pd, load(kbuf, c), _NN)
            dvk = _dot(pd, rhs, _TN).astype(BF16)
            vbuf[part(i, c)] = dvk[:, :dh].reshape(STEP, PIECE, dh)
            kbuf[part(i, c)] = dvk[:, dh:].reshape(STEP, PIECE, dh)
            return acc + jnp.where(top, o, dq)

        od_s[i] = lax.fori_loop(0, steps, second_pass, jnp.zeros((ROWS, dh), F32))
        refill(i, 1, 3)

    started = QUEUE + 3 * REFILL * (nh - TURN)
    assert sum(GROUPS[:pl.cdiv(started, 2 * PIECES)]) <= TURN * bph

    tail_in.wait()
    db_b = ((1.0 - gate) * go).astype(BF16)
    pre = _dot(x_b, w1_v[...], _NN)
    act_b = jnp.maximum(pre, 0.0).astype(BF16)
    b_out = _dot(act_b, w2_v[...], _NN)
    slope = jnp.where(pre > 0.0, 1.0, jnp.where(pre == 0.0, 0.5, 0.0))
    dpre_b = (_dot(db_b, w2_v[...], _NT) * slope).astype(BF16)
    dw2_v[...] = _dot(act_b, db_b, _TN).astype(BF16).reshape(dw2_v.shape)
    dw1_v[...] = _dot(x_b, dpre_b, _TN).astype(BF16).reshape(dw1_v.shape)

    start_cache_out(started, started + 2 * REFILL)

    def from_heads(r0):
        row = lax.broadcasted_iota(jnp.int32, (ROWS, dh), 0)
        cols = []
        for hq in range(HQ):
            h, r = divmod(hq, rep)
            col = jnp.zeros((ROWS, dh), F32)
            for b in range(nb):
                col = jnp.where(row == b, od_s[b * hkv + h, r0 + r:r0 + r + 1, :], col)
            cols.append(col)
        return jnp.concatenate(cols, axis=1).astype(BF16)

    o_b = from_heads(0)
    dq_b = from_heads(rep)
    a_out = _dot(o_b, wo_v[...], _NN)
    dz = jnp.sum(go * (a_out - b_out), axis=-1, keepdims=True) * gate * (1.0 - gate)
    out = gate * a_out + (1.0 - gate) * b_out
    dx = _dot(dq_b, wq_v[...], _NT) + _dot(dpre_b, w1_v[...], _NT) + dz * gw
    out_v[...] = out[:nb].astype(BF16)
    dx_v[...] = dx[:nb].astype(BF16)
    dgw_v[...] = jnp.sum(dz * x, axis=0, keepdims=True).astype(BF16).reshape(-1)
    start_cache_out(started + 2 * REFILL, started + 4 * REFILL)
    dwo_v[...] = _dot(o_b, da_b, _TN).astype(BF16).reshape(dwo_v.shape)
    start_cache_out(started + 4 * REFILL, started + 6 * REFILL)
    dwq_v[...] = _dot(x_b, dq_b, _TN).astype(BF16).reshape(dwq_v.shape)

    small_out = [
        pltpu.make_async_copy(src, dst, out_sem.at[1])
        for src, dst in ((out_v, out_hbm), (dx_v, dx_hbm), (dgw_v, dgw_hbm))
    ]
    for copy in small_out:
        copy.start()
    last_run = (len(runs) - 1) * PIECES
    start_cache_out(started + 6 * REFILL, last_run)

    weights = ((dwq_v, dwq_hbm), (dwo_v, dwo_hbm), (dw1_v, dw1_hbm), (dw2_v, dw2_hbm))

    def start_weight_out(w, j, rows, c, cols):
        buf, hbm = weights[w]
        idx = slice(None), pl.ds(pl.multiple_of(j * rows, rows), rows), pl.ds(c * cols, cols)
        pltpu.make_async_copy(buf.at[idx], hbm.at[idx], out_sem.at[2 + w]).start()

    @pl.loop(0, dwq_v.shape[1] // 8)
    def _(j):
        for c in range(2):
            start_weight_out(0, j, 8, c, dwq_v.shape[2] // 2)
            start_weight_out(2, 2 * j + c, 8, 0, dw1_v.shape[2])

    @pl.loop(0, dwo_v.shape[1] // 32)
    def _(j):
        start_weight_out(1, j, 32, 0, dwo_v.shape[2])

        @pl.when(j < dw2_v.shape[1] // 32)
        def _():
            start_weight_out(3, j, 32, 0, dw2_v.shape[2])

    start_cache_out(last_run, last_run + PIECES)

    for copy in small_out:
        copy.wait()
    for w, (buf, hbm) in enumerate(weights):
        pltpu.make_async_copy(buf, hbm, out_sem.at[2 + w]).wait()
    pltpu.make_async_copy(kbuf.at[pl.ds(0, dk_hbm.shape[0])], dk_hbm, out_sem.at[0]).wait()


@jax.jit
def pallas_gated_mix__gqa_block_cached__dense_activation_relu__decode_kernel(
    A_x: jax.Array,
    A_k_cache: jax.Array,
    A_v_cache: jax.Array,
    A_wq: jax.Array,
    A_wo: jax.Array,
    B_x: jax.Array,
    B_w1: jax.Array,
    B_w2: jax.Array,
    gate_w: jax.Array,
    grad_out: jax.Array,
):
    del B_x
    nb, hkv, sk, dh = A_k_cache.shape
    nh = nb * hkv
    rows = (nb, A_x.shape[-1])
    bph = sk // (PIECE * PIECES)
    cache = (nh * bph, PIECES, PIECE, dh)
    slots = ((nh + 1) * bph, PIECES, PIECE, dh)
    scores = (sk // (STEP * PIECE), ROWS, STEP * PIECE)
    weights = (A_wq, A_wo, B_w1, B_w2)
    split = [(n, w.shape[0] // n, w.shape[1]) for n, w in zip(SPLITS, weights)]
    assert sum(GROUPS) == cache[0]
    assert split[0][1] % 8 == 0 and split[2][1] == 2 * split[0][1]
    assert split[1][1] % 32 == 0 and split[3][1] % 32 == 0 and split[3][1] <= split[1][1]

    out_shapes = (rows, rows, cache, cache, *split, gate_w.shape)
    hbm = pl.BlockSpec(memory_space=pltpu.HBM)
    outs = pl.pallas_call(
        functools.partial(_kernel, heads=nh),
        out_shape=tuple(jax.ShapeDtypeStruct(s, BF16) for s in out_shapes),
        in_specs=[hbm] * 9,
        out_specs=(hbm,) * 9,
        scratch_shapes=[
            *(pltpu.VMEM(s, BF16) for s in (slots, slots, *(w.shape for w in weights), *split)),
            *(pltpu.VMEM(s, BF16) for s in (rows, rows, gate_w.shape) * 2),
            *(pltpu.VMEM((nh, ROWS, dh), F32) for _ in range(3)),
            *(pltpu.VMEM(scores, F32) for _ in range(3)),
            pltpu.SemaphoreType.DMA,
        ],
        compiler_params=pltpu.CompilerParams(vmem_limit_bytes=112 * 1024 * 1024),
    )(
        A_x.reshape(rows), A_k_cache.reshape(cache), A_v_cache.reshape(cache),
        *weights, gate_w, grad_out.reshape(rows),
    )
    like = (A_x, A_x, A_k_cache, A_v_cache, *weights, gate_w)
    return tuple(o.reshape(a.shape) for o, a in zip(outs, like))
```
